```python
import os as _os
_os.environ.setdefault("JAX_PLATFORMS", "cpu")
import jax
import jax.numpy as jnp

def _softmax(x, axis=-1):
    return jax.nn.softmax(x, axis=axis)
def _gelu(x):
    return jax.nn.gelu(x, approximate=True)
def _silu(x):
    return jax.nn.silu(x)
def _sigmoid(x):
    return jax.nn.sigmoid(x)
def _layernorm(x, axis=-1, eps=1e-5):
    m = jnp.mean(x, axis=axis, keepdims=True)
    v = jnp.var(x, axis=axis, keepdims=True)
    return (x - m) / jnp.sqrt(v + eps)
def _scatter_add(tgt, idx, src, axis=0):
    return tgt.at[idx].add(src)
def _segment_sum(src, seg, n):
    return jax.ops.segment_sum(src, seg, n)
class _Rng:
    def __init__(self, key):
        self._k = key
    def _next(self):
        self._k, sub = jax.random.split(self._k)
        return sub
    def normal(self, shape):
        return jax.random.normal(self._next(), shape, dtype=jnp.bfloat16)
    def randint(self, lo, hi, shape):
        return jax.random.randint(self._next(), shape, lo, hi, dtype=jnp.int32)
    def uniform(self, shape, lo=0.0, hi=1.0):
        return jax.random.uniform(self._next(), shape, jnp.bfloat16, lo, hi)
    def permutation(self, n):
        return jax.random.permutation(self._next(), n)


kernel_name = 'standalone__mha_softmax__near_ridge'

def setup_inputs():
    _rng = _Rng(jax.random.key(int.from_bytes(__import__("os").urandom(4), "little")))
    _w = (lambda a: (lambda t: t.astype(jnp.bfloat16) if jnp.issubdtype(t.dtype, jnp.floating) else t)(jnp.asarray(a)))
    B, H, Sq, Sk, D = 8, 32, 304, 2048, 128
    return {
        "q": _w((lambda *s: _rng.normal(s) * 0.4)(B, H, Sq, D)),
        "k": _w((lambda *s: _rng.normal(s) * 0.4)(B, H, Sk, D)),
        "v": _w((lambda *s: _rng.normal(s) * 0.05)(B, H, Sk, D)),
    }

def reference(q, k, v):
    scale = q.shape[-1] ** -0.5
    scores = jnp.einsum("bhqd,bhkd->bhqk", q, k) * scale
    p = _softmax(scores, axis=-1)
    return jnp.einsum("bhqk,bhkd->bhqd", p, v)
```

```python
import functools

import jax
import jax.numpy as jnp
import jax.experimental.pallas as pl
import jax.experimental.pallas.tpu as pltpu
import numpy as np

_LOG2E = 1.4426950408889634
_LANES = 128

_GROUP = 16
_SLOTS = 16
_OUT_CHUNK = 8
_KEY_BLOCK = 512


def _fold_lanes(x, op):
    r = x[:, :_LANES]
    for t in range(1, x.shape[1] // _LANES):
        r = op(r, x[:, t * _LANES:(t + 1) * _LANES])
    return r


def _attend_one_head(q, k_ref, v_ref, scale_log2e):
    sq, d = q.shape
    sk = k_ref.shape[0]
    q = (q.astype(jnp.float32) * scale_log2e).astype(q.dtype)
    m_run = l_run = acc = None
    for j in range(sk // _KEY_BLOCK):
        rows = pl.ds(j * _KEY_BLOCK, _KEY_BLOCK)
        s = jax.lax.dot_general(q, k_ref[rows, :], (((1,), (1,)), ((), ())),
                                preferred_element_type=jnp.float32)
        m_blk = jnp.max(_fold_lanes(s, jnp.maximum), axis=-1, keepdims=True)
        m_blk = jnp.broadcast_to(m_blk, (sq, _LANES))
        m_new = m_blk if m_run is None else jnp.maximum(m_run, m_blk)
        p = jnp.exp2(s - jnp.concatenate([m_new] * (_KEY_BLOCK // _LANES), axis=1))
        l_blk = _fold_lanes(p, jnp.add)
        pv = jnp.dot(p.astype(v_ref.dtype), v_ref[rows, :], preferred_element_type=jnp.float32)
        if m_run is None:
            l_run, acc = l_blk, pv
        else:
            alpha = jnp.exp2(m_run - m_new)
            l_run = l_run * alpha + l_blk
            acc = acc * alpha + pv
        m_run = m_new
    l = jnp.sum(l_run, axis=-1, keepdims=True)
    return acc * pltpu.reciprocal(l, approx=True)


def _mha_kernel(q_hbm, k_hbm, v_hbm, o_hbm, q_buf, k_buf, v_buf, o_buf, in_sem, out_sem):
    n_heads, _, d = q_hbm.shape
    n_iter = n_heads // _GROUP
    banks = _SLOTS // _GROUP
    scale_log2e = np.float32(d ** -0.5 * _LOG2E)

    def in_copies(h, slot):
        return (pltpu.make_async_copy(q_hbm.at[h], q_buf.at[slot], in_sem.at[0, slot]),
                pltpu.make_async_copy(k_hbm.at[h], k_buf.at[slot], in_sem.at[1, slot]),
                pltpu.make_async_copy(v_hbm.at[h], v_buf.at[slot], in_sem.at[2, slot]))

    def out_copy(chunk):
        heads = pl.ds(chunk * _OUT_CHUNK, _OUT_CHUNK)
        return pltpu.make_async_copy(o_buf.at[heads], o_hbm.at[heads], out_sem.at[chunk])

    for h in range(_SLOTS):
        for cp in in_copies(h, h):
            cp.start()

    def body(it, carry):
        base = (it % banks) * _GROUP
        prev_base = ((it + banks - 1) % banks) * _GROUP
        for g in range(_GROUP):
            h = it * _GROUP + g
            slot = base + g
            for cp in in_copies(h, slot):
                cp.wait()

            refill = (h - 1) + _SLOTS
            if g > 0:
                refill_slot, refill_ok = slot - 1, refill < n_heads
            else:
                refill_slot = prev_base + _GROUP - 1
                refill_ok = jnp.logical_and(it > 0, refill < n_heads)

            @pl.when(refill_ok)
            def _():
                for cp in in_copies(refill, refill_slot):
                    cp.start()

            if g % _OUT_CHUNK == 0:
                if g > 0:
                    out_copy(h // _OUT_CHUNK - 1).start()
                else:
                    @pl.when(it > 0)
                    def _():
                        out_copy(h // _OUT_CHUNK - 1).start()

            out = _attend_one_head(q_buf[slot], k_buf.at[slot], v_buf.at[slot], scale_log2e)
            o_buf[h] = out.astype(o_buf.dtype)
        return carry

    jax.lax.fori_loop(0, n_iter, body, 0)

    n_chunks = n_heads // _OUT_CHUNK
    out_copy(n_chunks - 1).start()
    for chunk in range(n_chunks):
        out_copy(chunk).wait()


@jax.jit
def pallas_standalone__mha_softmax__near_ridge_kernel(
    q: jax.Array,
    k: jax.Array,
    v: jax.Array,
):
    b, h, sq, d = q.shape
    sk = k.shape[2]
    n_heads = b * h
    assert n_heads % _SLOTS == 0 and _SLOTS % _GROUP == 0 and _GROUP % _OUT_CHUNK == 0
    assert sk % _KEY_BLOCK == 0 and d == _LANES

    out = pl.pallas_call(
        _mha_kernel,
        in_specs=[pl.BlockSpec(memory_space=pl.ANY)] * 3,
        out_specs=pl.BlockSpec(memory_space=pl.ANY),
        out_shape=jax.ShapeDtypeStruct((n_heads, sq, d), q.dtype),
        scratch_shapes=[
            pltpu.VMEM((_SLOTS, sq, d), q.dtype),
            pltpu.VMEM((_SLOTS, sk, d), k.dtype),
            pltpu.VMEM((_SLOTS, sk, d), v.dtype),
            pltpu.VMEM((n_heads, sq, d), q.dtype),
            pltpu.SemaphoreType.DMA((3, _SLOTS)),
            pltpu.SemaphoreType.DMA((n_heads // _OUT_CHUNK,)),
        ],
        compiler_params=pltpu.CompilerParams(
            vmem_limit_bytes=110 * 1024 * 1024,
            disable_bounds_checks=True,
            flags={"XLA_TPU_RESCHEDULE_DMA_DONES": True},
        ),
    )(q.reshape(n_heads, sq, d), k.reshape(n_heads, sk, d), v.reshape(n_heads, sk, d))
    return out.reshape(b, h, sq, d)
```

```python
import jax
import jax.numpy as jnp
import jax.experimental.pallas as pl
import jax.experimental.pallas.tpu as pltpu
import numpy as np

_LOG2E = 1.4426950408889634
_LANES = 128

_GROUP = 16
_AHEAD = 8
_OUT_CHUNK = 8
_KEY_BLOCK = 512


def _lane_tiles(x):
    return [x[:, t * _LANES:(t + 1) * _LANES] for t in range(x.shape[1] // _LANES)]


def _max_tiles(x):
    tiles = _lane_tiles(x)
    r = tiles[0]
    for t in tiles[1:]:
        r = jnp.maximum(r, t)
    return r


def _attend_one_head(q, k_ref, v_ref, wait_for_v):
    sq, d = q.shape
    sk = k_ref.shape[0]
    q = (q.astype(jnp.float32) * np.float32(d ** -0.5 * _LOG2E)).astype(q.dtype)
    m_run = l_run = acc = None
    for j in range(sk // _KEY_BLOCK):
        keys = pl.ds(j * _KEY_BLOCK, _KEY_BLOCK)
        s = jax.lax.dot_general(q, k_ref[keys, :], (((1,), (1,)), ((), ())),
                                preferred_element_type=jnp.float32)
        m_blk = jnp.max(_max_tiles(s), axis=-1, keepdims=True)
        m_blk = jnp.broadcast_to(m_blk, (sq, _LANES))
        m_new = m_blk if j == 0 else jnp.maximum(m_run, m_blk)
        p = jnp.exp2(s - jnp.concatenate([m_new] * (_KEY_BLOCK // _LANES), axis=1))

        p_tiles = _lane_tiles(p)
        if j == 0:
            l_run = p_tiles.pop(0)
        else:
            alpha = jnp.exp2(m_run - m_new)
            l_run = l_run * alpha
        for t in p_tiles:
            l_run = l_run + t

        if j == 0:
            wait_for_v()
        pv = jnp.dot(p.astype(v_ref.dtype), v_ref[keys, :], preferred_element_type=jnp.float32)
        acc = pv if j == 0 else pv + acc * alpha
        m_run = m_new
    l = jnp.sum(l_run, axis=-1, keepdims=True)
    return acc * pltpu.reciprocal(l, approx=True)


def _mha_kernel(q_hbm, k_hbm, v_hbm, o_hbm, q_buf, k_buf, v_buf, o_buf,
                in_sem, out_sem, tail_sem):
    n_heads = q_hbm.shape[0]
    n_iter = n_heads // _GROUP
    n_chunks = n_heads // _OUT_CHUNK

    def q_copy(h, slot):
        return pltpu.make_async_copy(q_hbm.at[h], q_buf.at[slot], in_sem.at[0, slot])

    def k_copy(h, slot):
        return pltpu.make_async_copy(k_hbm.at[h], k_buf.at[slot], in_sem.at[1, slot])

    def v_copy(h, slot):
        return pltpu.make_async_copy(v_hbm.at[h], v_buf.at[slot], in_sem.at[2, slot])

    def chunk_copy(chunk):
        heads = pl.ds(chunk * _OUT_CHUNK, _OUT_CHUNK)
        return pltpu.make_async_copy(o_buf.at[heads], o_hbm.at[heads], out_sem.at[chunk])

    def tail_copy(i):
        h = n_heads - _OUT_CHUNK + i
        return pltpu.make_async_copy(o_buf.at[h], o_hbm.at[h], tail_sem.at[i])

    for h in range(_AHEAD):
        q_copy(h, h).start()
        k_copy(h, h).start()
        v_copy(h, h).start()

    def body(it, carry):
        for g in range(_GROUP):
            h = it * _GROUP + g
            q_copy(h, g).wait()
            k_copy(h, g).wait()

            @pl.when(h + _AHEAD < n_heads)
            def _():
                slot = (g + _AHEAD) % _GROUP
                q_copy(h + _AHEAD, slot).start()
                k_copy(h + _AHEAD, slot).start()
                v_copy(h + _AHEAD, slot).start()

            if g % _OUT_CHUNK == 0:
                if g > 0:
                    chunk_copy(h // _OUT_CHUNK - 1).start()
                else:
                    @pl.when(it > 0)
                    def _():
                        chunk_copy(h // _OUT_CHUNK - 1).start()
            if g > _GROUP - _OUT_CHUNK:
                @pl.when(it == n_iter - 1)
                def _():
                    tail_copy(g - 1 - (_GROUP - _OUT_CHUNK)).start()

            q = q_buf[g]
            if g > 0:
                q = jnp.where(it < 0, o_buf[h - 1], q)
            out = _attend_one_head(q, k_buf.at[g], v_buf.at[g], lambda: v_copy(h, g).wait())
            o_buf[h] = out.astype(o_buf.dtype)
        return carry

    jax.lax.fori_loop(0, n_iter, body, 0)

    tail_copy(_OUT_CHUNK - 1).start()
    for chunk in range(n_chunks - 1):
        chunk_copy(chunk).wait()
    for i in range(_OUT_CHUNK):
        tail_copy(i).wait()


@jax.jit
def pallas_standalone__mha_softmax__near_ridge_kernel(
    q: jax.Array,
    k: jax.Array,
    v: jax.Array,
):
    b, h, sq, d = q.shape
    sk = k.shape[2]
    n_heads = b * h
    assert n_heads % _GROUP == 0 and _GROUP % _OUT_CHUNK == 0 and _AHEAD < _GROUP
    assert sk % _KEY_BLOCK == 0 and d == _LANES

    out = pl.pallas_call(
        _mha_kernel,
        in_specs=[pl.BlockSpec(memory_space=pl.ANY)] * 3,
        out_specs=pl.BlockSpec(memory_space=pl.ANY),
        out_shape=jax.ShapeDtypeStruct((n_heads, sq, d), q.dtype),
        scratch_shapes=[
            pltpu.VMEM((_GROUP, sq, d), q.dtype),
            pltpu.VMEM((_GROUP, sk, d), k.dtype),
            pltpu.VMEM((_GROUP, sk, d), v.dtype),
            pltpu.VMEM((n_heads, sq, d), q.dtype),
            pltpu.SemaphoreType.DMA((3, _GROUP)),
            pltpu.SemaphoreType.DMA((n_heads // _OUT_CHUNK - 1,)),
            pltpu.SemaphoreType.DMA((_OUT_CHUNK,)),
        ],
        compiler_params=pltpu.CompilerParams(
            vmem_limit_bytes=100 * 1024 * 1024,
            disable_bounds_checks=True,
            disable_semaphore_checks=True,
            flags={"XLA_TPU_RESCHEDULE_DMA_DONES": True},
        ),
    )(q.reshape(n_heads, sq, d), k.reshape(n_heads, sk, d), v.reshape(n_heads, sk, d))
    return out.reshape(b, h, sq, d)
```
